```python
import os as _os
_os.environ.setdefault("JAX_PLATFORMS", "cpu")
import jax
import jax.numpy as jnp

def _softmax(x, axis=-1):
    return jax.nn.softmax(x, axis=axis)
def _gelu(x):
    return jax.nn.gelu(x, approximate=True)
def _silu(x):
    return jax.nn.silu(x)
def _sigmoid(x):
    return jax.nn.sigmoid(x)
def _layernorm(x, axis=-1, eps=1e-5):
    m = jnp.mean(x, axis=axis, keepdims=True)
    v = jnp.var(x, axis=axis, keepdims=True)
    return (x - m) / jnp.sqrt(v + eps)
def _scatter_add(tgt, idx, src, axis=0):
    return tgt.at[idx].add(src)
def _segment_sum(src, seg, n):
    return jax.ops.segment_sum(src, seg, n)
class _Rng:
    def __init__(self, key):
        self._k = key
    def _next(self):
        self._k, sub = jax.random.split(self._k)
        return sub
    def normal(self, shape):
        return jax.random.normal(self._next(), shape, dtype=jnp.bfloat16)
    def randint(self, lo, hi, shape):
        return jax.random.randint(self._next(), shape, lo, hi, dtype=jnp.int32)
    def uniform(self, shape, lo=0.0, hi=1.0):
        return jax.random.uniform(self._next(), shape, jnp.bfloat16, lo, hi)
    def permutation(self, n):
        return jax.random.permutation(self._next(), n)


kernel_name = 'concat_heads__mha_block__linear_attn_block__prompt'

def setup_inputs():
    _rng = _Rng(jax.random.key(int.from_bytes(__import__("os").urandom(4), "little")))
    _w = (lambda a: (lambda t: t.astype(jnp.bfloat16) if jnp.issubdtype(t.dtype, jnp.floating) else t)(jnp.asarray(a)))
    def _A_setup():
        B, S, D, H = 1, 2048, 1024, 32
        return {
            "x": _w((lambda *s: _rng.normal(s) * 0.2)(B, S, D)),
            "wqkv": _w((lambda *s: _rng.normal(s) * 0.2)(D, 3 * D)),
            "wo": _w((lambda *s: _rng.normal(s) * 0.05)(D, D)),
        }
    _A_in = _A_setup()

    def _B_setup():
        B, S, D = 1, 2048, 1024
        return {
            "x": _w((lambda *s: _rng.normal(s) * 0.05)(B, S, D)),
            "wqkv": _w((lambda *s: _rng.normal(s) * 1.6)(D, 3 * D)),
            "wo": _w((lambda *s: _rng.normal(s) * 0.1)(D, D)),
        }
    _B_in = _B_setup()

    return {
        "A_x": _A_in["x"],
        "A_wqkv": _A_in["wqkv"],
        "A_wo": _A_in["wo"],
        "B_x": _B_in["x"],
        "B_wqkv": _B_in["wqkv"],
        "B_wo": _B_in["wo"],
    }

def reference(A_x, A_wqkv, A_wo, B_x, B_wqkv, B_wo):
    def _A_ref(x, wqkv, wo):
        B, S, D = x.shape
        H = 32
        Dh = D // H
        qkv = (lambda x, *d: x.transpose(*d))((x @ wqkv).reshape(B, S, 3, H, Dh), 2, 0, 3, 1, 4)
        q, k, v = qkv[0], qkv[1], qkv[2]
        scores = jnp.einsum("bhqd,bhkd->bhqk", q, k) * (Dh ** -0.5)
        p = _softmax(scores, axis=-1)
        o = jnp.einsum("bhqk,bhkd->bhqd", p, v)
        return (lambda x, *d: x.transpose(*d))(o, 0, 2, 1, 3).reshape(B, S, D) @ wo

    def _B_ref(x, wqkv, wo):
        B, S, D = x.shape
        H = 32; Dh = D // H
        qkv = (lambda x, *d: x.transpose(*d))((x @ wqkv).reshape(B, S, 3, H, Dh), 2, 0, 3, 1, 4)
        q, k, v = qkv[0], qkv[1], qkv[2]
        phi = lambda t: jnp.where(t > 0, t + 1, jnp.exp(t)) + 1e-6
        pq, pk = phi(q), phi(k)
        kv = jnp.einsum("bhsd,bhse->bhde", pk, v)
        z = jnp.einsum("bhsd->bhd", pk)
        num = jnp.einsum("bhqd,bhde->bhqe", pq, kv)
        den = jnp.einsum("bhqd,bhd->bhq", pq, z)[..., None] + 1e-6
        o = num / den
        return (lambda x, *d: x.transpose(*d))(o, 0, 2, 1, 3).reshape(B, S, D) @ wo

    a = _A_ref(A_x, A_wqkv, A_wo)
    b = _B_ref(B_x, B_wqkv, B_wo)
    return jnp.concatenate([a, b], axis=-1)
```

```python
import jax
import jax.numpy as jnp
from jax import lax
import jax.experimental.pallas as pl
import jax.experimental.pallas.tpu as pltpu

S = 2048
D = 1024
H = 32
DH = D // H
BM = 512
BQ = 512
CK = 128
LOG2E = 1.4426950408889634

bf16 = jnp.bfloat16
f32 = jnp.float32
u32 = jnp.uint32


def _tree(xs, op):
    xs = list(xs)
    while len(xs) > 1:
        xs = [op(xs[i], xs[i + 1]) if i + 1 < len(xs) else xs[i]
              for i in range(0, len(xs), 2)]
    return xs[0]


def _rows8(x, op):
    return _tree([x[i:i + 8] for i in range(0, x.shape[0], 8)], op)


def _dot(a, b):
    return jnp.dot(a, b, preferred_element_type=f32)


def _phi(t):
    return jnp.where(t > 0, t + 1.0, jnp.exp(t)) + 1e-6


def _kernel(ax_hbm, aw_hbm, awo_hbm, bx_hbm, bw_hbm, bwo_hbm, out_hbm,
            ax, aw, awo, bx, bw, bwo,
            qT, kk, vT, oT, sb0, sb1, kv, kvz, ostage, isem, osem):
    def wcopy(src, dst, c, i):
        cols = pl.ds(c * D, D)
        return pltpu.make_async_copy(src.at[:, cols], dst.at[:, cols], isem.at[i])

    def xcopy(src, dst, r, i):
        rows = pl.ds(r * BM, BM)
        return pltpu.make_async_copy(src.at[rows], dst.at[rows], isem.at[i])

    nb = S // BM
    bx_c = [xcopy(bx_hbm, bx, r, r) for r in range(nb)]
    bwk_c = wcopy(bw_hbm, bw, 1, nb)
    bwv_c = wcopy(bw_hbm, bw, 2, nb + 1)
    bwq_c = wcopy(bw_hbm, bw, 0, nb + 2)
    bwo_c = pltpu.make_async_copy(bwo_hbm, bwo, isem.at[nb + 3])
    ax_c = pltpu.make_async_copy(ax_hbm, ax, isem.at[nb + 4])
    aw_c = pltpu.make_async_copy(aw_hbm, aw, isem.at[nb + 5])
    awo_c = pltpu.make_async_copy(awo_hbm, awo, isem.at[nb + 6])
    for c in [bx_c[0], bwk_c, bwv_c] + bx_c[1:] + [bwq_c, bwo_c, ax_c, aw_c, awo_c]:
        c.start()

    def ocopy(slot, r, col):
        return pltpu.make_async_copy(
            ostage.at[slot], out_hbm.at[pl.ds(r * BM, BM), pl.ds(col, D)],
            osem.at[slot])

    z8 = jnp.zeros((8, D), f32)
    for r in range(nb):
        bx_c[r].wait()
        if r == 0:
            bwk_c.wait()
        x = bx[pl.ds(r * BM, BM), :]
        pk = _phi(_dot(x, bw[:, pl.ds(D, D)]))
        z8 = z8 + _rows8(pk, jnp.add)
        pkT = pk.astype(bf16).T
        if r == 0:
            bwv_c.wait()
        v = _dot(x, bw[:, pl.ds(2 * D, D)]).astype(bf16)
        for g in range(D // 128):
            t = _dot(pkT[g * 128:(g + 1) * 128], v[:, g * 128:(g + 1) * 128])
            if r == 0:
                kv[g] = t
            else:
                kv[g] += t
    z = jnp.sum(z8, axis=0, keepdims=True)
    ri = lax.broadcasted_iota(jnp.int32, (128, 128), 0) // DH
    ci = lax.broadcasted_iota(jnp.int32, (128, 128), 1) // DH
    same_head = ri == ci
    for g in range(D // 128):
        zcol = jnp.broadcast_to(z[:, g * 128:(g + 1) * 128], (128, 128)).T
        kvz[g, :, pl.ds(0, 128)] = jnp.where(same_head, kv[g], 0.0).astype(bf16)
        kvz[g, :, pl.ds(128, 128)] = jnp.where(same_head, zcol, 0.0).astype(bf16)

    bwq_c.wait()
    bwo_c.wait()
    for r in range(nb):
        x = bx[pl.ds(r * BM, BM), :]
        pq = _phi(_dot(x, bw[:, pl.ds(0, D)])).astype(bf16)
        os_ = []
        for g in range(D // 128):
            nd = _dot(pq[:, g * 128:(g + 1) * 128], kvz[g])
            os_.append((nd[:, :128] / (nd[:, 128:] + 1e-6)).astype(bf16))
        o = jnp.concatenate(os_, axis=1)
        res = _dot(o, bwo[...]).astype(bf16)
        if r >= 2:
            ocopy(r % 2, r - 2, D).wait()
        ostage[r % 2] = res
        ocopy(r % 2, r, D).start()

    ax_c.wait()
    aw_c.wait()

    def proj(r, carry):
        r0 = pl.multiple_of(r * BM, BM)
        x = ax[pl.ds(r0, BM), :]
        k = _dot(x, aw[:, pl.ds(D, D)]).astype(bf16)
        for h in range(H):
            kk[h, pl.ds(pl.multiple_of(r * (BM // 2), BM // 2), BM // 2), :] = (
                pltpu.bitcast(k[:, h * DH:(h + 1) * DH], u32))
        q = (_dot(x, aw[:, pl.ds(0, D)]) * (DH ** -0.5 * LOG2E)).astype(bf16)
        qT[:, pl.ds(r0, BM)] = pltpu.bitcast(q.T, u32)
        v = _dot(x, aw[:, pl.ds(2 * D, D)]).astype(bf16)
        vT[:, pl.ds(r0, BM)] = pltpu.bitcast(v.T, u32)
        return carry

    lax.fori_loop(0, nb, proj, 0)
    awo_c.wait()

    nq = S // BQ
    hp = DH // 2

    def getq(h, qb):
        return pltpu.bitcast(
            qT[pl.ds(pl.multiple_of(h * hp, hp), hp),
               pl.ds(pl.multiple_of(qb * BQ, BQ), BQ)], bf16)

    def qk_chunk(h, r0, q, sb, m):
        kc = pltpu.bitcast(kk[h, pl.ds(r0 // 2, CK // 2), :], bf16)
        s = _dot(kc, q)
        sb[pl.ds(r0, CK), :] = s
        return jnp.maximum(m, _rows8(s, jnp.maximum))

    def pv_chunk(h, r0, sb, mb, l, acc):
        p = jnp.exp2(sb[pl.ds(r0, CK), :] - mb)
        l = l + _rows8(p, jnp.add)
        v = pltpu.bitcast(
            vT[pl.ds(pl.multiple_of(h * hp, hp), hp), pl.ds(r0, CK)], bf16)
        return l, acc + _dot(v, p.astype(bf16))

    neg = jnp.full((8, BQ), -jnp.inf, f32)

    def head(h, qb, mcur, sc, sn):
        nxt = jnp.minimum(qb * H + h + 1, nq * H - 1)
        hn = nxt % H
        qn = getq(hn, nxt // H)
        mb = jnp.max(mcur, axis=0, keepdims=True)
        m, l, acc = neg, jnp.zeros((8, BQ), f32), jnp.zeros((DH, BQ), f32)
        for c in range(S // CK):
            m = qk_chunk(hn, c * CK, qn, sn, m)
            l, acc = pv_chunk(h, c * CK, sc, mb, l, acc)
        lt = jnp.sum(l, axis=0, keepdims=True)
        oT[pl.ds(pl.multiple_of(h * hp, hp), hp), :] = pltpu.bitcast(
            (acc / lt).astype(bf16), u32)
        return m

    q0 = getq(0, 0)
    m0 = lax.fori_loop(
        0, S // CK,
        lambda c, m: qk_chunk(0, pl.multiple_of(c * CK, CK), q0, sb0, m), neg)

    def qblock(qb, m):
        def pair(i, m):
            m = head(2 * i, qb, m, sb0, sb1)
            return head(2 * i + 1, qb, m, sb1, sb0)

        m = lax.fori_loop(0, H // 2, pair, m)
        o = pltpu.bitcast(oT[...], bf16).T
        res = _dot(o, awo[...]).astype(bf16)
        slot = qb % 2
        ocopy(slot, 0, 0).wait()
        ostage[slot] = res
        ocopy(slot, qb, 0).start()
        return m

    lax.fori_loop(0, nq, qblock, m0)
    ocopy(0, 0, 0).wait()
    ocopy(1, 0, 0).wait()


@jax.jit
def pallas_concat_heads__mha_block__linear_attn_block__prompt_kernel(
    A_x: jax.Array,
    A_wqkv: jax.Array,
    A_wo: jax.Array,
    B_x: jax.Array,
    B_wqkv: jax.Array,
    B_wo: jax.Array,
):
    any_spec = pl.BlockSpec(memory_space=pl.ANY)
    out = pl.pallas_call(
        _kernel,
        out_shape=jax.ShapeDtypeStruct((S, 2 * D), bf16),
        in_specs=[any_spec] * 6,
        out_specs=any_spec,
        scratch_shapes=[
            pltpu.VMEM((S, D), bf16),
            pltpu.VMEM((D, 3 * D), bf16),
            pltpu.VMEM((D, D), bf16),
            pltpu.VMEM((S, D), bf16),
            pltpu.VMEM((D, 3 * D), bf16),
            pltpu.VMEM((D, D), bf16),
            pltpu.VMEM((D // 2, S), u32),
            pltpu.VMEM((H, S // 2, DH), u32),
            pltpu.VMEM((D // 2, S), u32),
            pltpu.VMEM((D // 2, BQ), u32),
            pltpu.VMEM((S, BQ), f32),
            pltpu.VMEM((S, BQ), f32),
            pltpu.VMEM((D // 128, 128, 128), f32),
            pltpu.VMEM((D // 128, 128, 256), bf16),
            pltpu.VMEM((2, BM, D), bf16),
            pltpu.SemaphoreType.DMA((S // BM + 7,)),
            pltpu.SemaphoreType.DMA((2,)),
        ],
        compiler_params=pltpu.CompilerParams(vmem_limit_bytes=110 * 1024 * 1024),
        name="mha_linattn",
    )(A_x.reshape(S, D), A_wqkv, A_wo, B_x.reshape(S, D), B_wqkv, B_wo)
    return out.reshape(1, S, 2 * D)
```

```python
import jax
import jax.numpy as jnp
from jax import lax
import jax.experimental.pallas as pl
import jax.experimental.pallas.tpu as pltpu

S = 2048
D = 1024
H = 32
DH = D // H
BM = 512
BQ = 512
CK = 128
UN = 10
NO = 4
KS0 = (0, 128, 256, 512, 768, 1024)
LOG2E = 1.4426950408889634

bf16 = jnp.bfloat16
f32 = jnp.float32
u32 = jnp.uint32


def _rows8(x, op):
    xs = [x[i:i + 8] for i in range(0, x.shape[0], 8)]
    while len(xs) > 1:
        xs = [op(xs[i], xs[i + 1]) if i + 1 < len(xs) else xs[i]
              for i in range(0, len(xs), 2)]
    return xs[0]


def _dot(a, b):
    return jnp.dot(a, b, preferred_element_type=f32)


def _phi(t):
    return jnp.where(t > 0, t + 1.0, jnp.exp(t)) + 1e-6


def _pack(x):
    return pltpu.bitcast(x, u32)


def _unpack(x):
    return pltpu.bitcast(x, bf16)


def _kernel(ax_hbm, aw_hbm, awo_hbm, bx_hbm, bw_hbm, bwo_hbm, out_hbm,
            ax, aw, awo, bx, bw, bwo,
            qT, kk, vT, oT, sb0, sb1, zcol, mfold, pqn, ostage, isem, osem):
    nb = S // BM
    ng = D // 128
    n0 = len(KS0) - 1

    copies = []

    def fetch(src, dst):
        c = pltpu.make_async_copy(src, dst, isem.at[len(copies)])
        copies.append(c)
        c.start()
        return c

    def fetch_w(src, dst, c):
        return fetch(src.at[:, pl.ds(c * D, D)], dst.at[:, pl.ds(c * D, D)])

    def fetch_first(j):
        ks = pl.ds(KS0[j], KS0[j + 1] - KS0[j])
        return (fetch(bx_hbm.at[pl.ds(0, BM), ks], bx.at[pl.ds(0, BM), ks]),
                fetch(bw_hbm.at[ks, pl.ds(D, D)], bw.at[ks, pl.ds(D, D)]))

    first = [fetch_first(j) for j in range(n0)]
    z8 = jnp.zeros((8, D), f32)
    for r in range(nb):
        rows = pl.ds(r * BM, BM)
        if r == 0:
            k = None
            for j in range(n0):
                first[j][0].wait()
                first[j][1].wait()
                if j == 2:
                    x1 = fetch(bx_hbm.at[pl.ds(BM, BM)], bx.at[pl.ds(BM, BM)])
                if j == n0 - 1:
                    rest = pl.ds(2 * BM, S - 2 * BM)
                    x2 = fetch(bx_hbm.at[rest], bx.at[rest])
                ks = pl.ds(KS0[j], KS0[j + 1] - KS0[j])
                t = _dot(bx[rows, ks], bw[ks, pl.ds(D, D)])
                k = t if k is None else k + t
        else:
            if r == 1:
                x1.wait()
                b_rest = [fetch_w(bw_hbm, bw, 2), fetch(bwo_hbm, bwo),
                          fetch_w(bw_hbm, bw, 0)]
            if r == 2:
                x2.wait()
                a_all = [fetch(ax_hbm, ax), fetch(aw_hbm, aw), fetch(awo_hbm, awo)]
            if r == nb - 1:
                for c in b_rest:
                    c.wait()
            k = _dot(bx[rows, :], bw[:, pl.ds(D, D)])
        pk = _phi(k)
        z8 = z8 + _rows8(pk, jnp.add)
        qT[:, rows] = _pack(pk.astype(bf16).T)
    z = jnp.sum(z8, axis=0, keepdims=True)
    for g in range(ng):
        zcol[pl.ds(g * 128, 128), :] = jnp.broadcast_to(
            z[:, g * 128:(g + 1) * 128], (128, 128)).T
    gm = _dot(_unpack(qT[...]), bx[...]).astype(bf16)
    same_head = (lax.broadcasted_iota(jnp.int32, (128, 128), 0) // DH
                 == lax.broadcasted_iota(jnp.int32, (128, 128), 1) // DH)

    kvs = []
    for r in range(nb):
        rows = pl.ds(r * BM, BM)
        if r == 1:
            for c in a_all:
                c.wait()
        pqT = _phi(_dot(bx[rows, :], bw[:, pl.ds(0, D)])).astype(bf16).T
        if r == 0:
            for g in range(ng):
                kv = _dot(gm[g * 128:(g + 1) * 128],
                          bw[:, pl.ds(2 * D + g * 128, 128)])
                kvs.append(jnp.where(same_head, kv, 0.0).astype(bf16))
        if r == 1:
            for g in range(ng):
                gs = pl.ds(g * 128, 128)
                mfold[gs, :] = _dot(kvs[g], bwo[gs, :]).astype(bf16)
        parts = []
        for h in range(H):
            ph = pqT[h * DH:(h + 1) * DH].astype(f32)
            zh = zcol[pl.ds(h * DH, DH), :]
            zh = jnp.concatenate([zh] * (BM // 128), axis=1)
            den = jnp.sum(_rows8(ph * zh, jnp.add), axis=0, keepdims=True) + 1e-6
            parts.append((ph * (1.0 / den)).astype(bf16))
        pqn[pl.ds(r * (BM // 2), BM // 2), :] = _pack(
            jnp.concatenate(parts, axis=0).T)

    for r in range(nb):
        rows = pl.ds(r * BM, BM)
        x = ax[rows, :]
        k = _dot(x, aw[:, pl.ds(D, D)]).astype(bf16)
        for h in range(H):
            kk[h, pl.ds(r * (BM // 2), BM // 2), :] = _pack(k[:, h * DH:(h + 1) * DH])
        q = (_dot(x, aw[:, pl.ds(0, D)]) * (DH ** -0.5 * LOG2E)).astype(bf16)
        qT[:, rows] = _pack(q.T)
        v = _dot(x, aw[:, pl.ds(2 * D, D)]).astype(bf16)
        vT[:, rows] = _pack(v.T)

    hp = DH // 2
    nc = S // CK
    no = D // NO
    neg = jnp.full((8, BQ), -jnp.inf, f32)

    def hrows(h):
        return pl.ds(pl.multiple_of(h * hp, hp), hp)

    def put(qb, j):
        cols = pl.ds(j * no, no)
        return pltpu.make_async_copy(
            ostage.at[:, cols],
            out_hbm.at[pl.ds(pl.multiple_of(qb * BQ, BQ), BQ), cols], osem.at[j])

    def qblock(qb, carry):
        qcols = pl.ds(pl.multiple_of(qb * BQ, BQ), BQ)
        zero = (qb >> 20) * 8

        def getq(h):
            return _unpack(qT[hrows(h), qcols])

        def qk_chunk(h, c, q, sb, m):
            s = _dot(_unpack(kk[h, pl.ds(c * (CK // 2), CK // 2), :]), q)
            sb[pl.ds(pl.multiple_of(c * CK + zero, 8), CK), :] = s
            return jnp.maximum(m, _rows8(s, jnp.maximum))

        def head(h, mcur, sc, sn, filler=None):
            if filler is None:
                qn = getq(h + 1)
            mb = jnp.max(mcur, axis=0, keepdims=True)
            m, l, acc = neg, jnp.zeros((8, BQ), f32), jnp.zeros((DH, BQ), f32)
            p = None
            for c in range(nc + 1):
                p_prev = p
                if c < nc:
                    if filler is None:
                        m = qk_chunk(h + 1, c, qn, sn, m)
                    else:
                        filler(c)
                    e = jnp.exp2(sc[pl.ds(c * CK, CK), :] - mb)
                    l = l + _rows8(e, jnp.add)
                    p = e.astype(bf16)
                if c > 0:
                    vc = _unpack(vT[hrows(h), pl.ds((c - 1) * CK, CK)])
                    acc = acc + _dot(vc, p_prev)
            o = acc / jnp.sum(l, axis=0, keepdims=True)
            oT[hrows(h), :] = _pack(o.astype(bf16))
            return m

        m = neg
        q0 = getq(0)
        for c in range(nc):
            m = qk_chunk(0, c, q0, sb0, m)

        def heads(i, m):
            for u in range(0, UN, 2):
                m = head(i * UN + u, m, sb0, sb1)
                m = head(i * UN + u + 1, m, sb1, sb0)
            return m

        m = lax.fori_loop(0, (H - 2) // UN, heads, m)

        @pl.when(qb > 0)
        def _():
            for j in range(2 * NO):
                put(qb - 1, j).wait()

        m = head(H - 2, m, sb0, sb1)

        kd = D - 128
        o_main = _unpack(oT[pl.ds(0, kd // 2), :]).T
        part = []

        def filler(c):
            if c % (nc // NO) == 0:
                j = c // (nc // NO)
                part.append(_dot(o_main, awo[pl.ds(0, kd), pl.ds(j * no, no)]))

        head(H - 1, m, sb1, sb0, filler)
        o_last = _unpack(oT[pl.ds(kd // 2, 64), :]).T
        pb = _unpack(pqn[pl.ds(pl.multiple_of(qb * (BQ // 2), BQ // 2), BQ // 2), :])
        for j in range(NO):
            cols = pl.ds(j * no, no)
            ostage[:, pl.ds(D + j * no, no)] = _dot(pb, mfold[:, cols]).astype(bf16)
            put(qb, NO + j).start()
            res = part[j] + _dot(o_last, awo[pl.ds(kd, 128), cols])
            ostage[:, cols] = res.astype(bf16)
            put(qb, j).start()
        return carry

    lax.fori_loop(0, S // BQ, qblock, 0)
    for j in range(2 * NO):
        put(S // BQ - 1, j).wait()


@jax.jit
def pallas_concat_heads__mha_block__linear_attn_block__prompt_kernel(
    A_x: jax.Array,
    A_wqkv: jax.Array,
    A_wo: jax.Array,
    B_x: jax.Array,
    B_wqkv: jax.Array,
    B_wo: jax.Array,
):
    any_spec = pl.BlockSpec(memory_space=pl.ANY)
    out = pl.pallas_call(
        _kernel,
        out_shape=jax.ShapeDtypeStruct((S, 2 * D), bf16),
        in_specs=[any_spec] * 6,
        out_specs=any_spec,
        scratch_shapes=[
            pltpu.VMEM((S, D), bf16),
            pltpu.VMEM((D, 3 * D), bf16),
            pltpu.VMEM((D, D), bf16),
            pltpu.VMEM((S, D), bf16),
            pltpu.VMEM((D, 3 * D), bf16),
            pltpu.VMEM((D, D), bf16),
            pltpu.VMEM((D // 2, S), u32),
            pltpu.VMEM((H, S // 2, DH), u32),
            pltpu.VMEM((D // 2, S), u32),
            pltpu.VMEM((D // 2, BQ), u32),
            pltpu.VMEM((S, BQ), f32),
            pltpu.VMEM((S, BQ), f32),
            pltpu.VMEM((D, 128), f32),
            pltpu.VMEM((D, D), bf16),
            pltpu.VMEM((S // 2, D), u32),
            pltpu.VMEM((BQ, 2 * D), bf16),
            pltpu.SemaphoreType.DMA((2 * (len(KS0) - 1) + 8,)),
            pltpu.SemaphoreType.DMA((2 * NO,)),
        ],
        compiler_params=pltpu.CompilerParams(vmem_limit_bytes=110 * 1024 * 1024),
        name="mha_linattn",
    )(A_x.reshape(S, D), A_wqkv, A_wo, B_x.reshape(S, D), B_wqkv, B_wo)
    return out.reshape(1, S, 2 * D)
```
